```python
import jax
import jax.numpy as jnp

def _softmax(x, axis=-1):
    return jax.nn.softmax(x, axis=axis)
def _gelu(x):
    return jax.nn.gelu(x, approximate=True)
def _silu(x):
    return jax.nn.silu(x)
def _sigmoid(x):
    return jax.nn.sigmoid(x)
def _layernorm(x, axis=-1, eps=1e-5):
    m = jnp.mean(x, axis=axis, keepdims=True)
    v = jnp.var(x, axis=axis, keepdims=True)
    return (x - m) / jnp.sqrt(v + eps)
def _scatter_add(tgt, idx, src, axis=0):
    return tgt.at[idx].add(src)
def _segment_sum(src, seg, n):
    return jax.ops.segment_sum(src, seg, n)
class _Rng:
    def __init__(self, key):
        self._k = key
    def _next(self):
        self._k, sub = jax.random.split(self._k)
        return sub
    def normal(self, shape):
        return jax.random.normal(self._next(), shape, dtype=jnp.bfloat16)
    def randint(self, lo, hi, shape):
        return jax.random.randint(self._next(), shape, lo, hi, dtype=jnp.int32)
    def uniform(self, shape, lo=0.0, hi=1.0):
        return jax.random.uniform(self._next(), shape, jnp.bfloat16, lo, hi)
    def permutation(self, n):
        return jax.random.permutation(self._next(), n)


kernel_name = 'standalone__fft_conv__vision'

def setup_inputs():
    _rng = _Rng(jax.random.key(int.from_bytes(__import__("os").urandom(4), "little")))
    _w = (lambda a: (lambda t: t.astype(jnp.bfloat16) if jnp.issubdtype(t.dtype, jnp.floating) else t)(jnp.asarray(a)))
    H = W = 224
    C = 96
    K = 7
    return {
        "x": _w((lambda *s: _rng.normal(s) * 0.05)(1, H, W, C)),
        "w": _w((lambda *s: _rng.normal(s) * 0.05)(K, K, C, C)),
    }

def reference(x, w):
    B, H, W, C = x.shape
    K = w.shape[0]
    wp = jnp.pad(w, ((0, H - K), (0, W - K), (0, 0), (0, 0)))
    Xf = (lambda x, axes=(-2,-1): jnp.fft.rfft2(x.astype(jnp.float32), axes=axes))(x, axes=(1, 2))
    Wf = (lambda x, axes=(-2,-1): jnp.fft.rfft2(x.astype(jnp.float32), axes=axes))(wp, axes=(0, 1))
    Yf = jnp.einsum('bhwi,hwio->bhwo', Xf, Wf)
    y = (lambda x, s, axes=(-2,-1): jnp.fft.irfft2(x, s=s, axes=axes).astype(jnp.bfloat16))(Yf, (H, W), axes=(1, 2))
    return y
```

```python
import math
import jax
import jax.numpy as jnp
import numpy as np
import jax.experimental.pallas as pl
import jax.experimental.pallas.tpu as pltpu

H = W = 224
C = 96
TW, LW, NTW = 34, 28, 8
TH, LH, NTH = 20, 14, 16
NF = TW // 2
R1 = TW * NTW
S3 = 36
NT = (((1,), (1,)), ((), ()))


def _consts():
    th = 2 * np.pi * (np.arange(NF) + 0.5) / TW
    q = np.arange(TW)
    blk = np.zeros((TW, TW))
    blk[0::2] = np.cos(np.outer(th, q))
    blk[1::2] = -np.sin(np.outer(th, q))
    fa = np.zeros((4 * TW, 128), np.float32)
    fb = np.zeros((4 * TW, 128), np.float32)
    for t in range(4):
        fa[t * TW:(t + 1) * TW, LW * t:LW * t + TW] = blk
        fb[t * TW:(t + 1) * TW, 10 + LW * t:10 + LW * t + TW] = blk
    qo = np.arange(6, TW) - 3
    g = np.zeros((2 * LW, 2 * S3), np.float32)
    sc = 2.0 / (TW * TH)
    for t in range(2):
        g[t * LW:(t + 1) * LW, t * S3:t * S3 + TW:2] = sc * np.cos(np.outer(qo, th))
        g[t * LW:(t + 1) * LW, t * S3 + 1:t * S3 + TW:2] = -sc * np.sin(np.outer(qo, th))
    k = np.arange(1, 4)
    cw = np.concatenate([np.cos(np.outer(th, k)), -np.sin(np.outer(th, k))], axis=1)
    return fa, fb, g, cw.astype(np.float32)


def _add(p, q):
    return (p[0] + q[0], p[1] + q[1])


def _sub(p, q):
    return (p[0] - q[0], p[1] - q[1])


def _scl(p, c):
    return (p[0] * c, p[1] * c)


def _add_i(p, q, sign):
    if sign > 0:
        return (p[0] - q[1], p[1] + q[0])
    return (p[0] + q[1], p[1] - q[0])


def _dft4(x, sign):
    t0, t1 = _add(x[0], x[2]), _sub(x[0], x[2])
    t2, t3 = _add(x[1], x[3]), _sub(x[1], x[3])
    return [_add(t0, t2), _add_i(t1, t3, sign), _sub(t0, t2), _add_i(t1, t3, -sign)]


def _dft5(x, sign):
    c1, c2 = math.cos(2 * math.pi / 5), math.cos(4 * math.pi / 5)
    s1, s2 = math.sin(2 * math.pi / 5), math.sin(4 * math.pi / 5)
    t1, t2 = _add(x[1], x[4]), _add(x[2], x[3])
    t3, t4 = _sub(x[1], x[4]), _sub(x[2], x[3])
    t5 = _add(t1, t2)
    t6 = _scl(_sub(t1, t2), (c1 - c2) / 2)
    t7 = _sub(x[0], _scl(t5, 0.25))
    a, b = _add(t7, t6), _sub(t7, t6)
    u = _add(_scl(t3, s1), _scl(t4, s2))
    v = _sub(_scl(t3, s2), _scl(t4, s1))
    return [_add(x[0], t5), _add_i(a, u, sign), _add_i(b, v, sign),
            _add_i(b, v, -sign), _add_i(a, u, -sign)]


def _dft20(get, emit, sign):
    a = [_dft4([get((5 * n1 + 4 * n2) % 20) for n1 in range(4)], sign) for n2 in range(5)]
    for k1 in range(4):
        o = _dft5([a[n2][k1] for n2 in range(5)], sign)
        for k2 in range(5):
            emit((5 * k1 + 16 * k2) % 20, o[k2])


def _kernel(x_hbm, w_ref, fa_ref, fb_ref, g_ref, cw_ref, y_hbm,
            xbuf, ybuf, z1, z2, z3, weo, wbuf, sem_in, sem_out):
    def in_copy(b):
        return pltpu.make_async_copy(x_hbm.at[pl.ds(b * LH, LH)], xbuf.at[b], sem_in.at[b])

    def out_copy(b):
        return pltpu.make_async_copy(ybuf.at[b], y_hbm.at[pl.ds(b * LH, LH)], sem_out.at[b])

    order = [NTH - 1] + list(range(NTH - 1))
    for b in order:
        in_copy(b).start()

    def fold(v):
        return [v[3], v[4] + v[2], v[5] + v[1], v[6] + v[0], v[4] - v[2], v[5] - v[1], v[6] - v[0]]
    for r in range(C // 16):
        rows = pl.ds(r * 16, 16)
        t = [fold([w_ref[a, b, rows, :].astype(jnp.float32) for b in range(7)]) for a in range(7)]
        for b in range(7):
            o = fold([t[a][b] for a in range(7)])
            for a in range(7):
                weo[a, b, rows, :] = o[a]
    z3[...] = jnp.zeros(z3.shape, jnp.float32)

    def wfwd_row(b, slot, hl):
        xr = xbuf[b, hl]
        wa = jnp.concatenate([xr[:, 218:224], xr[:, 0:122]], axis=1)
        wb = xr[:, 96:224]
        z1[slot, hl, pl.ds(0, 4 * TW), :] = jax.lax.dot_general(
            fa_ref[...], wa, NT, preferred_element_type=jnp.float32)
        z1[slot, hl, pl.ds(4 * TW, 4 * TW), :] = jax.lax.dot_general(
            fb_ref[...], wb, NT, preferred_element_type=jnp.float32)

    def slot_of(b):
        return jnp.where(b == NTH - 1, 3, b % 3)

    def fft_col(t, sp, sc, k):
        def get(p):
            s, hl = (sp, p + LH - 6) if p < 6 else (sc, p - 6)
            return (z1[s, hl, pl.ds(2 * k, NTW, stride=TW), :],
                    z1[s, hl, pl.ds(2 * k + 1, NTW, stride=TW), :])

        def emit(f, v):
            rows = pl.ds(pl.multiple_of(t * NTW, NTW), NTW)
            z2[k, f, 0, rows, :] = v[0]
            z2[k, f, 1, rows, :] = v[1]
        _dft20(get, emit, -1)

    def p1_w(b):
        in_copy(b).wait()
        s = slot_of(b)
        for hl in range(LH):
            wfwd_row(b, s, hl)

    def p1_f(t):
        sp, sc = slot_of((t + NTH - 1) % NTH), slot_of(t)
        for k in range(NF):
            fft_col(t, sp, sc, k)

    def p1_pro(i, c):
        p1_w((i + NTH - 1) % NTH)
        return c
    jax.lax.fori_loop(0, 2, p1_pro, 0)

    def p1_main(b, c):
        p1_w(b)
        p1_f(b - 1)
        return c
    jax.lax.fori_loop(1, NTH - 1, p1_main, 0)

    def p1_epi(t, c):
        p1_f(t)
        return c
    jax.lax.fori_loop(NTH - 2, NTH, p1_epi, 0)

    def gen_rows(k, slot, r):
        rows = pl.ds(r * 8, 8)
        cs = [cw_ref[k, j] for j in range(6)]
        u = []
        for a in range(7):
            re = weo[a, 0, rows, :] + weo[a, 1, rows, :] * cs[0] + weo[a, 2, rows, :] * cs[1] \
                + weo[a, 3, rows, :] * cs[2]
            im = weo[a, 4, rows, :] * cs[3] + weo[a, 5, rows, :] * cs[4] + weo[a, 6, rows, :] * cs[5]
            u.append((re, im))

        def put(f, v):
            wbuf[slot, f, 0, rows, :] = v[0]
            wbuf[slot, f, 1, rows, :] = v[1]
            wbuf[slot, f, 2, rows, :] = v[0] + v[1]
        e13 = _add(u[1], u[3])
        c2 = _add(u[0], u[2])
        put(0, _add(c2, e13))
        put(10, _sub(c2, e13))
        a5 = _sub(u[0], u[2])
        b5 = _sub(u[4], u[6])
        put(5, _add_i(a5, b5, -1))
        put(15, _add_i(a5, b5, 1))
        for f in range(1, 5):
            ph = 2 * math.pi * f / TH
            ev = _add(u[0], _scl(u[2], math.cos(2 * ph)))
            od = _add(_scl(u[1], math.cos(ph)), _scl(u[3], math.cos(3 * ph)))
            a0, a1 = _add(ev, od), _sub(ev, od)
            so = _add(_scl(u[4], math.sin(ph)), _scl(u[6], math.sin(3 * ph)))
            se = _scl(u[5], math.sin(2 * ph))
            b0, b1 = _add(so, se), _sub(so, se)
            put(f, _add_i(a0, b0, -1))
            put(TH - f, _add_i(a0, b0, 1))
            put(10 - f, _add_i(a1, b1, -1))
            put(10 + f, _add_i(a1, b1, 1))

    def prod(k, slot, f):
        xr, xi = z2[k, f, 0], z2[k, f, 1]
        p1 = jnp.dot(xr, wbuf[slot, f, 0], preferred_element_type=jnp.float32)
        p2 = jnp.dot(xi, wbuf[slot, f, 1], preferred_element_type=jnp.float32)
        p3 = jnp.dot(xr + xi, wbuf[slot, f, 2], preferred_element_type=jnp.float32)
        z2[k, f, 0] = p1 - p2
        z2[k, f, 1] = p3 - p1 - p2

    for r in range(C // 8):
        gen_rows(0, 0, r)

    def p2_body(k, c):
        kn = jnp.minimum(k + 1, NF - 1)
        s = k % 2
        for f in range(TH):
            prod(k, s, f)
            if f < C // 8:
                gen_rows(kn, 1 - s, f)
        return c
    jax.lax.fori_loop(0, NF, p2_body, 0)

    def ifft_col(t, slot, k):
        rows = pl.ds(pl.multiple_of(t * NTW, NTW), NTW)

        def get(f):
            return (z2[k, f, 0, rows, :], z2[k, f, 1, rows, :])

        def emit(p, v):
            if 3 <= p < 3 + LH:
                z3[slot, p - 3, pl.ds(2 * k, NTW, stride=S3), :] = v[0]
                z3[slot, p - 3, pl.ds(2 * k + 1, NTW, stride=S3), :] = v[1]
        _dft20(get, emit, 1)

    def winv_row(t, slot, hl):
        parts = [jnp.dot(g_ref[...], z3[slot, hl, pl.ds(2 * S3 * j, 2 * S3), :],
                         preferred_element_type=jnp.float32) for j in range(4)]
        ybuf[t, hl] = jnp.concatenate(parts, axis=0).astype(jnp.bfloat16).T

    def p3_i(t):
        for k in range(NF):
            ifft_col(t, t % 2, k)

    def p3_w(t):
        for hl in range(LH):
            winv_row(t, t % 2, hl)
        out_copy(t).start()

    def p3_pro(t, c):
        p3_i(t)
        return c
    jax.lax.fori_loop(0, 1, p3_pro, 0)

    def p3_main(t, c):
        p3_i(t)
        p3_w(t - 1)
        return c
    jax.lax.fori_loop(1, NTH, p3_main, 0)
    p3_w(NTH - 1)
    for b in range(NTH):
        out_copy(b).wait()


@jax.jit
def pallas_standalone__fft_conv__vision_kernel(x: jax.Array, w: jax.Array):
    fa, fb, g, cw = _consts()
    xt = jnp.transpose(x.reshape(H, W, C), (0, 2, 1))
    vm = pl.BlockSpec(memory_space=pltpu.VMEM)
    yt = pl.pallas_call(
        _kernel,
        out_shape=jax.ShapeDtypeStruct((H, C, W), jnp.bfloat16),
        in_specs=[pl.BlockSpec(memory_space=pl.ANY), vm, vm, vm, vm,
                  pl.BlockSpec(memory_space=pltpu.SMEM)],
        out_specs=pl.BlockSpec(memory_space=pl.ANY),
        scratch_shapes=[
            pltpu.VMEM((NTH, LH, C, W), jnp.bfloat16),
            pltpu.VMEM((NTH, LH, C, W), jnp.bfloat16),
            pltpu.VMEM((4, LH, R1, C), jnp.float32),
            pltpu.VMEM((NF, TH, 2, NTH * NTW, C), jnp.float32),
            pltpu.VMEM((2, LH, NTW * S3, C), jnp.float32),
            pltpu.VMEM((7, 7, C, C), jnp.float32),
            pltpu.VMEM((2, TH, 3, C, C), jnp.float32),
            pltpu.SemaphoreType.DMA((NTH,)),
            pltpu.SemaphoreType.DMA((NTH,)),
        ],
        compiler_params=pltpu.CompilerParams(vmem_limit_bytes=120 << 20),
    )(xt, w, fa, fb, g, cw)
    return jnp.transpose(yt, (0, 2, 1)).reshape(1, H, W, C)
```

```python
import math
import jax
import jax.numpy as jnp
import numpy as np
import jax.experimental.pallas as pl
import jax.experimental.pallas.tpu as pltpu

H = W = 224
C = 96
TW, LW, NTW = 34, 28, 8
TH, LH, NTH = 20, 14, 16
NF = TW // 2
R1 = TW * NTW
R3 = 312
NT = (((1,), (1,)), ((), ()))


def _consts():
    th = 2 * np.pi * (np.arange(NF) + 0.5) / TW
    q = np.arange(TW)
    blk = np.zeros((TW, TW))
    blk[0::2] = np.cos(np.outer(th, q))
    blk[1::2] = -np.sin(np.outer(th, q))
    fa = np.zeros((4 * TW, 128), np.float32)
    fb = np.zeros((4 * TW, 128), np.float32)
    for t in range(4):
        wa = (LW * t - 6 + q) % W
        fa[t * TW:(t + 1) * TW, np.where(wa >= 218, wa - 96, wa)] = blk
        wb = LW * (t + 4) - 6 + q
        fb[t * TW:(t + 1) * TW, np.where(wb >= 128, wb - 128, wb)] = blk
    qo = np.arange(6, TW) - 3
    g1 = np.zeros((LW, TW))
    sc = 2.0 / (TW * TH)
    g1[:, 0::2] = sc * np.cos(np.outer(qo, th))
    g1[:, 1::2] = -sc * np.sin(np.outer(qo, th))
    g = np.zeros((2 * LW, 80), np.float32)
    for t in range(2):
        g[t * LW:(t + 1) * LW, 40 * t:40 * t + 32] = g1[:, :32]
        g[t * LW:(t + 1) * LW, 40 * t + 38:40 * t + 40] = g1[:, 32:]
    k = np.arange(1, 4)
    cw = np.concatenate([np.cos(np.outer(th, k)), -np.sin(np.outer(th, k))], axis=1)
    cw = np.concatenate([cw, np.zeros((1, 6))], axis=0)
    return fa, fb, g, cw.astype(np.float32)


LAG1 = 1


def _pack(a, b):
    return pltpu.pack_elementwise([a, b], packed_dtype=jnp.bfloat16)


def _add(p, q):
    return (p[0] + q[0], p[1] + q[1])


def _sub(p, q):
    return (p[0] - q[0], p[1] - q[1])


def _scl(p, c):
    return (p[0] * c, p[1] * c)


def _add_i(p, q, sign):
    if sign > 0:
        return (p[0] - q[1], p[1] + q[0])
    return (p[0] + q[1], p[1] - q[0])


def _dft4(x, sign):
    t0, t1 = _add(x[0], x[2]), _sub(x[0], x[2])
    t2, t3 = _add(x[1], x[3]), _sub(x[1], x[3])
    return [_add(t0, t2), _add_i(t1, t3, sign), _sub(t0, t2), _add_i(t1, t3, -sign)]


def _dft5(x, sign):
    c1, c2 = math.cos(2 * math.pi / 5), math.cos(4 * math.pi / 5)
    s1, s2 = math.sin(2 * math.pi / 5), math.sin(4 * math.pi / 5)
    t1, t2 = _add(x[1], x[4]), _add(x[2], x[3])
    t3, t4 = _sub(x[1], x[4]), _sub(x[2], x[3])
    t5 = _add(t1, t2)
    t6 = _scl(_sub(t1, t2), (c1 - c2) / 2)
    t7 = _sub(x[0], _scl(t5, 0.25))
    a, b = _add(t7, t6), _sub(t7, t6)
    u = _add(_scl(t3, s1), _scl(t4, s2))
    v = _sub(_scl(t3, s2), _scl(t4, s1))
    return [_add(x[0], t5), _add_i(a, u, sign), _add_i(b, v, sign),
            _add_i(b, v, -sign), _add_i(a, u, -sign)]


def _dft20(get, emit, sign):
    a = [_dft4([get((5 * n1 + 4 * n2) % 20) for n1 in range(4)], sign) for n2 in range(5)]
    for k1 in range(4):
        o = _dft5([a[n2][k1] for n2 in range(5)], sign)
        for k2 in range(5):
            emit((5 * k1 + 16 * k2) % 20, o[k2])


def _kernel(x_hbm, w_ref, fa_ref, fb_ref, g_ref, cw_ref, y_hbm,
            xy, zs, z2, weo, wa, wb, sem_in, sem_out):
    xu = x_hbm.bitcast(jnp.uint32)
    yu = y_hbm.bitcast(jnp.uint32)

    def in_copy(b):
        return pltpu.make_async_copy(xu.at[pl.ds(b * LH, LH)], xy.at[pl.ds(b * LH, LH)], sem_in.at[b])

    def out_copy(b):
        return pltpu.make_async_copy(xy.at[pl.ds(b * LH, LH)], yu.at[pl.ds(b * LH, LH)], sem_out.at[b])

    for b in [NTH - 1] + list(range(NTH - 1)):
        in_copy(b).start()

    never = jax.lax.broadcasted_iota(jnp.int32, (8, C), 1) < cw_ref[NF, 0].astype(jnp.int32)

    def tie(v, deps):
        for d in deps:
            v = jnp.where(never, d, v)
        return v

    def fold(v):
        return [v[3], v[4] + v[2], v[5] + v[1], v[6] + v[0], v[4] - v[2], v[5] - v[1], v[6] - v[0]]
    for r in range(C // 16):
        rows = pl.ds(r * 16, 16)
        t = [fold([w_ref[a, b, rows, :].astype(jnp.float32) for b in range(7)]) for a in range(7)]
        for b in range(7):
            o = fold([t[a][b] for a in range(7)])
            for a in range(7):
                weo[a, b, rows, :] = o[a]

    def gen(k, wdst):
        cs = [cw_ref[k, j] for j in range(6)]
        for r in range(C // 16):
            us = []
            for par in range(2):
                rows = pl.ds(r * 16 + par, 8, stride=2)
                u = []
                for a in range(7):
                    re = weo[a, 0, rows, :] + weo[a, 1, rows, :] * cs[0] \
                        + weo[a, 2, rows, :] * cs[1] + weo[a, 3, rows, :] * cs[2]
                    im = weo[a, 4, rows, :] * cs[3] + weo[a, 5, rows, :] * cs[4] \
                        + weo[a, 6, rows, :] * cs[5]
                    u.append((re, im))
                us.append(u)
            orow = pl.ds(r * 8, 8)
            for f in range(5):
                deps = yield
                res = []
                for u in us:
                    u0 = (tie(u[0][0], deps), u[0][1])
                    u4 = (tie(u[4][0], deps), u[4][1])
                    if f == 0:
                        e13, c2 = _add(u[1], u[3]), _add(u0, u[2])
                        a5, b5 = _sub(u0, u[2]), _sub(u4, u[6])
                        res.append({0: _add(c2, e13), 10: _sub(c2, e13),
                                    5: _add_i(a5, b5, -1), 15: _add_i(a5, b5, 1)})
                    else:
                        ph = 2 * math.pi * f / TH
                        ev = _add(u0, _scl(u[2], math.cos(2 * ph)))
                        od = _add(_scl(u[1], math.cos(ph)), _scl(u[3], math.cos(3 * ph)))
                        a0, a1 = _add(ev, od), _sub(ev, od)
                        so = _add(_scl(u4, math.sin(ph)), _scl(u[6], math.sin(3 * ph)))
                        se = _scl(u[5], math.sin(2 * ph))
                        b0, b1 = _add(so, se), _sub(so, se)
                        res.append({f: _add_i(a0, b0, -1), TH - f: _add_i(a0, b0, 1),
                                    10 - f: _add_i(a1, b1, -1), 10 + f: _add_i(a1, b1, 1)})
                for ff in res[0]:
                    v0, v1 = res[0][ff], res[1][ff]
                    wdst[ff, 0, orow, :] = _pack(v0[0], v1[0])
                    wdst[ff, 1, orow, :] = _pack(v0[1], v1[1])
                    wdst[ff, 2, orow, :] = _pack(v0[0] + v0[1], v1[0] + v1[1])

    def run_gen(g, n, deps):
        for _ in range(n):
            try:
                g.send(deps)
            except StopIteration:
                return

    z2[0:10, :, :, 0:NTW, :] = jnp.zeros((10, TH, 2, NTW, C), jnp.float32)
    g0 = gen(0, wa)
    next(g0)
    run_gen(g0, 64, ())

    def wfwd_row(src, dst):
        xr = pltpu.bitcast(xy[src], jnp.bfloat16)
        va = jnp.concatenate([xr[:, 0:122], xr[:, 218:224]], axis=1)
        vb = jnp.concatenate([xr[:, 128:224], xr[:, 96:128]], axis=1)
        ra = jax.lax.dot_general(fa_ref[...], va, NT, preferred_element_type=jnp.float32)
        rb = jax.lax.dot_general(fb_ref[...], vb, NT, preferred_element_type=jnp.float32)
        zs[dst, pl.ds(0, 4 * TW), :] = ra
        zs[dst, pl.ds(4 * TW, 4 * TW), :] = rb
        return [ra[:8], rb[:8]]

    def fft_col(t, k, deps=()):
        base = t * LH
        rows = pl.ds(pl.multiple_of(t * NTW + NTW, NTW), NTW)

        def get(p):
            re = zs[base + p, pl.ds(2 * k, NTW, stride=TW), :]
            return (tie(re, deps) if p == 0 else re,
                    zs[base + p, pl.ds(2 * k + 1, NTW, stride=TW), :])

        def emit(f, v):
            z2[k, f, 0, rows, :] = v[0]
            z2[k, f, 1, rows, :] = v[1]
        _dft20(get, emit, -1)

    in_copy(NTH - 1).wait()
    in_copy(0).wait()

    def p1_pro(i, c):
        for j in range(10):
            wfwd_row((10 * i + j + H - 6) % H, 10 * i + j)
        return c
    jax.lax.fori_loop(0, 2, p1_pro, 0)

    def p1_main(t, c):
        @pl.when(t < NTH - 2)
        def _():
            in_copy(t + 1).wait()
        deps = {}
        for i in range(NF):
            if i < LH:
                deps[i + LAG1] = wfwd_row(t * LH + LH + i, t * LH + TH + i)
            fft_col(t, i, deps.get(i, ()))
        return c
    jax.lax.fori_loop(0, NTH - 1, p1_main, 0)
    for k in range(NF):
        fft_col(NTH - 1, k)

    def prod(k, wsrc, f):
        def wl(g):
            return pltpu.bitcast(wsrc[f, g], jnp.bfloat16)
        xr, xi = z2[k, f, 0, NTW:, :], z2[k, f, 1, NTW:, :]
        p1 = jnp.dot(xr, wl(0), preferred_element_type=jnp.float32)
        p2 = jnp.dot(xi, wl(1), preferred_element_type=jnp.float32)
        p3 = jnp.dot(xr + xi, wl(2), preferred_element_type=jnp.float32)
        z2[k, f, 0, NTW:, :] = p1 - p2
        z2[k, f, 1, NTW:, :] = p3 - p1 - p2
        return [p1[0:8]]

    def p2_half(off, ws, wd):
        def body(j, c):
            k = 2 * j + off
            g = gen(jnp.minimum(k + 1, NF - 1), wd)
            next(g)
            for f in range(TH):
                d = prod(k, ws, f)
                if f >= 1:
                    run_gen(g, 2, d)
            return c
        return body

    def p2_outer(j, c):
        jax.lax.fori_loop(j, j + 1, p2_half(0, wa, wb), 0)
        jax.lax.fori_loop(j, jnp.minimum(j + 1, NF // 2), p2_half(1, wb, wa), 0)
        return c
    jax.lax.fori_loop(0, NF // 2 + 1, p2_outer, 0)

    def ifft_col(t, k, deps=()):
        base = t * LH
        rows = pl.ds(pl.multiple_of(t * NTW + NTW, NTW), NTW)

        def get(f):
            re = z2[k, f, 0, rows, :]
            return (tie(re, deps) if f == 0 else re, z2[k, f, 1, rows, :])

        def emit(p, v):
            if 3 <= p < 3 + LH:
                zs[base + p - 3, pl.ds(18 * k, NTW), :] = v[0]
                zs[base + p - 3, pl.ds(18 * k + 9, NTW), :] = v[1]
        _dft20(get, emit, 1)

    def winv_row(t, hl):
        src = t * LH - LH + hl
        rows = pl.ds(pl.multiple_of(t * NTW, NTW), NTW)
        out = []
        for j in range(4):
            rhs = jnp.concatenate([zs[src, pl.ds(2 * j + a + 9 * c0, n, stride=9), :]
                                   for a in range(2) for c0, n in ((0, 32), (26, 8))], axis=0)
            r = jnp.dot(g_ref[...], rhs, preferred_element_type=jnp.float32)
            for i in range(7):
                q = hl * 28 + 7 * j + i
                z2[q // 40, (q % 40) // 2, q % 2, rows, :] = r[8 * i:8 * i + 8]
            out.append(r[2 * LW - 8:])
        return out

    def xpose_row(t, hl):
        rows = pl.ds(pl.multiple_of(t * NTW - NTW, NTW), NTW)
        v = jnp.concatenate([z2[q // 40, (q % 40) // 2, q % 2, rows, :]
                             for q in range(hl * 28, hl * 28 + 28)], axis=0).astype(jnp.bfloat16).T
        xy[jnp.maximum(t - 2, 0) * LH + hl] = pltpu.bitcast(v, jnp.uint32)

    for k in range(NF):
        ifft_col(0, k)

    def p3_main(t, c):
        deps = {}
        for i in range(NF):
            if i < LH:
                deps[i + 2] = winv_row(t, i)
            ifft_col(t, i, deps.get(i, ()))
        for hl in range(LH):
            xpose_row(t, hl)

        @pl.when(t >= 2)
        def _():
            out_copy(t - 2).start()
        return c
    jax.lax.fori_loop(1, NTH, p3_main, 0)

    for hl in range(LH):
        winv_row(NTH, hl)
    for hl in range(LH):
        xpose_row(NTH, hl)
    out_copy(NTH - 2).start()
    for hl in range(LH):
        xpose_row(NTH + 1, hl)
    out_copy(NTH - 1).start()
    for b in range(NTH):
        out_copy(b).wait()


@jax.jit
def pallas_standalone__fft_conv__vision_kernel(x: jax.Array, w: jax.Array):
    fa, fb, g, cw = _consts()
    xt = jnp.transpose(x.reshape(H, W, C), (0, 2, 1))
    vm = pl.BlockSpec(memory_space=pltpu.VMEM)
    yt = pl.pallas_call(
        _kernel,
        out_shape=jax.ShapeDtypeStruct((H, C, W), jnp.bfloat16),
        in_specs=[pl.BlockSpec(memory_space=pl.ANY), vm, vm, vm, vm,
                  pl.BlockSpec(memory_space=pltpu.SMEM)],
        out_specs=pl.BlockSpec(memory_space=pl.ANY),
        scratch_shapes=[
            pltpu.VMEM((H, C // 2, W), jnp.uint32),
            pltpu.VMEM((H + 6, R3, C), jnp.float32),
            pltpu.VMEM((NF, TH, 2, (NTH + 1) * NTW, C), jnp.float32),
            pltpu.VMEM((7, 7, C, C), jnp.float32),
            pltpu.VMEM((TH, 3, C // 2, C), jnp.uint32),
            pltpu.VMEM((TH, 3, C // 2, C), jnp.uint32),
            pltpu.SemaphoreType.DMA((NTH,)),
            pltpu.SemaphoreType.DMA((NTH,)),
        ],
        compiler_params=pltpu.CompilerParams(vmem_limit_bytes=120 << 20),
    )(xt, w, fa, fb, g, cw)
    return jnp.transpose(yt, (0, 2, 1)).reshape(1, H, W, C)
```
